```python
import os as _os
_os.environ.setdefault('JAX_PLATFORMS', 'cpu')
import jax
import jax.numpy as jnp

def _softmax(x, axis=-1):
    return jax.nn.softmax(x, axis=axis)

def _gelu(x):
    return jax.nn.gelu(x, approximate=True)

def _silu(x):
    return jax.nn.silu(x)

def _sigmoid(x):
    return jax.nn.sigmoid(x)

def _layernorm(x, axis=-1, eps=1e-05):
    m = jnp.mean(x, axis=axis, keepdims=True)
    v = jnp.var(x, axis=axis, keepdims=True)
    return (x - m) / jnp.sqrt(v + eps)

def _scatter_add(tgt, idx, src, axis=0):
    return tgt.at[idx].add(src)

def _segment_sum(src, seg, n):
    return jax.ops.segment_sum(src, seg, n)

class _Rng:

    def __init__(self, key):
        self._k = key

    def _next(self):
        self._k, sub = jax.random.split(self._k)
        return sub

    def normal(self, shape):
        return jax.random.normal(self._next(), shape, dtype=jnp.bfloat16)

    def randint(self, lo, hi, shape):
        return jax.random.randint(self._next(), shape, lo, hi, dtype=jnp.int32)

    def uniform(self, shape, lo=0.0, hi=1.0):
        return jax.random.uniform(self._next(), shape, jnp.bfloat16, lo, hi)

    def permutation(self, n):
        return jax.random.permutation(self._next(), n)
kernel_name = 'adaLN_cond__mha_block__dense_activation_squared_relu__prompt'

def setup_inputs():
    _rng = _Rng(jax.random.key(int.from_bytes(__import__("os").urandom(4), "little")))
    _w = lambda a: (lambda t: t.astype(jnp.bfloat16) if jnp.issubdtype(t.dtype, jnp.floating) else t)(jnp.asarray(a))

    def _A_setup():
        B, S, D, H = (1, 2048, 512, 32)
        return {'x': _w((lambda *s: _rng.normal(s) * 0.05)(B, S, D)), 'wqkv': _w((lambda *s: _rng.normal(s) * 0.1)(D, 3 * D)), 'wo': _w((lambda *s: _rng.normal(s) * 0.05)(D, D))}
    _A_in = _A_setup()

    def _B_setup():
        B, S, D, F = (1, 2048, 512, 1792)
        return {'x': _w((lambda *s: _rng.normal(s) * 0.05)(B, S, D)), 'w1': _w((lambda *s: _rng.normal(s) * 0.05)(D, F)), 'b1': _w((lambda *s: _rng.normal(s) * 0.05)(F)), 'w2': _w((lambda *s: _rng.normal(s) * 0.05)(F, D)), 'b2': _w((lambda *s: _rng.normal(s) * 0.05)(D))}
    _B_in = _B_setup()
    return {'A_x': _A_in['x'], 'A_wqkv': _A_in['wqkv'], 'A_wo': _A_in['wo'], 'B_x': _B_in['x'], 'B_w1': _B_in['w1'], 'B_b1': _B_in['b1'], 'B_w2': _B_in['w2'], 'B_b2': _B_in['b2'], 'c': _w((lambda *s: _rng.normal(s) * 0.05)(1, 512) * 8.0), 'w_mod': _w((lambda *s: _rng.normal(s) * 0.05)(512, 6 * 512) * 512 ** (-0.5) * 8.0)}

def reference(A_x, A_wqkv, A_wo, B_x, B_w1, B_b1, B_w2, B_b2, c, w_mod):

    def _A_ref(x, wqkv, wo):
        B, S, D = x.shape
        H = 32
        Dh = D // H
        qkv = (lambda x, *d: x.transpose(*d))((x @ wqkv).reshape(B, S, 3, H, Dh), 2, 0, 3, 1, 4)
        q, k, v = (qkv[0], qkv[1], qkv[2])
        scores = jnp.einsum('bhqd,bhkd->bhqk', q, k) * Dh ** (-0.5)
        p = _softmax(scores, axis=-1)
        o = jnp.einsum('bhqk,bhkd->bhqd', p, v)
        return (lambda x, *d: x.transpose(*d))(o, 0, 2, 1, 3).reshape(B, S, D) @ wo

    def _B_ref(x, w1, b1, w2, b2):
        h = jnp.einsum('bsd,df->bsf', x, w1) + b1
        zero = jnp.zeros_like(h)
        r = jnp.where(h > zero, h, zero)
        h = r * r
        out = jnp.einsum('bsf,fd->bsd', h, w2) + b2
        return out
    x = A_x
    mod = (_silu(c) @ w_mod).reshape(c.shape[0], 6, 1, -1)
    sa, ca, ga, sb, cb, gb = (mod[:, 0].copy(), mod[:, 1].copy(), mod[:, 2].copy(), mod[:, 3].copy(), mod[:, 4].copy(), mod[:, 5].copy())
    h = _layernorm(x, axis=-1) * (1 + ca) + sa
    x = x + ga * _A_ref(h, A_wqkv, A_wo)
    h = _layernorm(x, axis=-1) * (1 + cb) + sb
    x = x + gb * _B_ref(h, B_w1, B_b1, B_w2, B_b2)
    return x
```

```python
import jax
import jax.numpy as jnp
import jax.experimental.pallas as pl
import jax.experimental.pallas.tpu as pltpu
from jax import lax

_S = 2048
_D = 512
_H = 32
_DH = 16
_F = 1792
_TQ = 512
_NT = _S // _TQ
_C = 128
_NC = _S // _C
_NI = _NT * _H
_EPS = 1e-5
_LOG2E = 1.4426950408889634

_bf = jnp.bfloat16
_f32 = jnp.float32
_i32 = jnp.int32
_NN = (((1,), (0,)), ((), ()))
_NTD = (((1,), (1,)), ((), ()))
_TN = (((0,), (0,)), ((), ()))


def _ldb(x):
    return pltpu.bitcast(x, _bf)


def _stb(x):
    return pltpu.bitcast(x, _i32)


def _dot(a, b, dims=_NN):
    return lax.dot_general(a, b, dims, preferred_element_type=_f32)


def _layernorm(x):
    m = jnp.mean(x, axis=-1, keepdims=True)
    xc = x - m
    v = jnp.mean(xc * xc, axis=-1, keepdims=True)
    return xc * lax.rsqrt(v + _EPS)


def _kernel(x_hbm, wqkv_hbm, wo_hbm, w1_hbm, b1_hbm, w2_hbm, b2_hbm, c_hbm, wm_hbm,
            out_hbm,
            x_v, wqkv_v, wo_v, w1_v, b1_v, w2_v, b2_v, c_v, wm_v,
            wqt_s, wvt_s, mod_s, k_s, qm_s, vt_s, sx_s, sy_s, ot_s, out_v, sems):
    def cp(src, dst, i):
        return pltpu.make_async_copy(src, dst, sems.at[i])

    c_cp = cp(c_hbm, c_v, 0)
    wma_cp = cp(wm_hbm.at[:, pl.ds(0, 2 * _D)], wm_v.at[:, pl.ds(0, 2 * _D)], 1)
    x_cps = [cp(x_hbm.at[0, pl.ds(b * _TQ, _TQ), :], x_v.at[pl.ds(b * _TQ, _TQ), :], 2 + b)
             for b in range(_NT)]
    wqkv_cp = cp(wqkv_hbm, wqkv_v, 6)
    wmb_cp = cp(wm_hbm.at[:, pl.ds(2 * _D, 4 * _D)], wm_v.at[:, pl.ds(2 * _D, 4 * _D)], 7)
    wo_cp = cp(wo_hbm, wo_v, 8)
    w1_cp = cp(w1_hbm, w1_v, 9)
    w2_cp = cp(w2_hbm, w2_v, 10)
    b1_cp = cp(b1_hbm, b1_v, 11)
    b2_cp = cp(b2_hbm, b2_v, 12)
    out_cps = [cp(out_v.at[pl.ds(t * _TQ, _TQ), :], out_hbm.at[0, pl.ds(t * _TQ, _TQ), :], 13 + t)
               for t in range(_NT)]

    c_cp.start()
    wma_cp.start()
    wqkv_cp.start()
    for b in range(_NT):
        x_cps[b].start()
    wmb_cp.start()
    wo_cp.start()
    w1_cp.start()
    w2_cp.start()
    b1_cp.start()
    b2_cp.start()

    qm_s[...] = jnp.zeros(qm_s.shape, _i32)

    c_cp.wait()
    cf = c_v[...].astype(_f32)
    sc = (cf * (1.0 / (1.0 + jnp.exp(-cf)))).astype(_bf)
    sc8 = jnp.broadcast_to(sc, (16, _D))
    wma_cp.wait()
    mod_s[:, pl.ds(0, 2 * _D)] = _dot(sc8, wm_v[:, pl.ds(0, 2 * _D)])[0:8]
    sa = mod_s[0:1, pl.ds(0, _D)]
    ca1 = 1.0 + mod_s[0:1, pl.ds(_D, _D)]

    wqkv_cp.wait()
    wqt_s[...] = _stb(wqkv_v[:, pl.ds(0, _D)].astype(_f32).T.astype(_bf))
    wvt_s[...] = _stb(wqkv_v[:, pl.ds(2 * _D, _D)].astype(_f32).T.astype(_bf))
    qscale = _DH ** -0.5 * _LOG2E
    for b in range(_NT):
        x_cps[b].wait()
        xb = x_v[pl.ds(b * _TQ, _TQ), :].astype(_f32)
        hb = (_layernorm(xb) * ca1 + sa).astype(_bf)
        kb = _dot(hb, wqkv_v[:, pl.ds(_D, _D)]).astype(_bf)
        for g in range(4):
            k_s[g, pl.ds(b * _TQ // 2, _TQ // 2), :] = _stb(kb[:, g * 128:(g + 1) * 128])
        qt = (_dot(_ldb(wqt_s[...]), hb, _NTD) * qscale).astype(_bf)
        vt = _dot(_ldb(wvt_s[...]), hb, _NTD).astype(_bf)
        for h in range(_H):
            qm_s[b * _H + h, pl.ds((h % 8) * _DH // 2, _DH // 2), :] = _stb(qt[h * _DH:(h + 1) * _DH, :])
            vt_s[h, :, pl.ds(b * _TQ, _TQ)] = _stb(vt[h * _DH:(h + 1) * _DH, :])

    def qk_chunk(n, s_ref, j):
        g = (n % _H) // 8
        s = _dot(_ldb(k_s[g, pl.ds(j * _C // 2, _C // 2), :]), _ldb(qm_s[n]))
        s_ref[pl.ds(j * _C, _C), :] = s
        return jnp.max(s.reshape(_C // 8, 8, _TQ), axis=0)

    def qk_only(n, s_ref):
        m8 = None
        for j in range(_NC):
            mm = qk_chunk(n, s_ref, j)
            m8 = mm if m8 is None else jnp.maximum(m8, mm)
        return m8

    def stage(n, nq, s_ref, m8_in):
        h = n % _H
        m = jnp.broadcast_to(jnp.max(m8_in, axis=0, keepdims=True), (8, _TQ))
        m8 = l8 = acc = None
        ps = {}
        for jj in range(_NC + 1):
            if jj < _NC:
                s = s_ref[pl.ds(jj * _C, _C), :]
                p = jnp.exp2(s.reshape(_C // 8, 8, _TQ) - m[None])
                ll = jnp.sum(p, axis=0)
                ps[jj] = p.reshape(_C, _TQ).astype(_bf)
                l8 = ll if l8 is None else l8 + ll
                mm = qk_chunk(nq, s_ref, jj)
                m8 = mm if m8 is None else jnp.maximum(m8, mm)
            if jj >= 1:
                j = jj - 1
                a = _dot(_ldb(vt_s[h, :, pl.ds(j * _C, _C)]), ps.pop(j))
                acc = a if acc is None else acc + a
        l = jnp.sum(l8, axis=0, keepdims=True)
        ot_s[n] = acc * (1.0 / l)
        return m8

    mx = qk_only(0, sx_s)
    my = qk_only(1, sy_s)

    def attn_body(i, carry):
        mx, my = carry
        n = 2 * i
        mx = stage(n, jnp.minimum(n + 2, _NI - 1), sx_s, mx)
        my = stage(n + 1, jnp.minimum(n + 3, _NI - 1), sy_s, my)
        return mx, my

    lax.fori_loop(0, _NI // 2, attn_body, (mx, my))

    wmb_cp.wait()
    mod_s[:, pl.ds(2 * _D, 4 * _D)] = _dot(sc8, wm_v[:, pl.ds(2 * _D, 4 * _D)])[0:8]
    wo_cp.wait()
    w1_cp.wait()
    w2_cp.wait()
    b1_cp.wait()
    b2_cp.wait()

    for t in range(_NT):
        ga = mod_s[0:1, pl.ds(2 * _D, _D)]
        sb = mod_s[0:1, pl.ds(3 * _D, _D)]
        cb1 = 1.0 + mod_s[0:1, pl.ds(4 * _D, _D)]
        gb = mod_s[0:1, pl.ds(5 * _D, _D)]
        ot = ot_s[pl.ds(t * _H, _H)].reshape(_D, _TQ)
        o = ot.T.astype(_bf)
        a = _dot(o, wo_v[...])
        x1 = x_v[pl.ds(t * _TQ, _TQ), :].astype(_f32) + ga * a
        h2 = (_layernorm(x1) * cb1 + sb).astype(_bf)
        hid = _dot(h2, w1_v[...]) + b1_v[...].astype(_f32)
        r = jnp.maximum(hid, 0.0)
        y = _dot((r * r).astype(_bf), w2_v[...]) + b2_v[...].astype(_f32)
        out_v[pl.ds(t * _TQ, _TQ), :] = (x1 + gb * y).astype(out_v.dtype)
        out_cps[t].start()
    for t in range(_NT):
        out_cps[t].wait()


@jax.jit
def pallas_adaLN_cond__mha_block__dense_activation_squared_relu__prompt_kernel(
    A_x: jax.Array,
    A_wqkv: jax.Array,
    A_wo: jax.Array,
    B_x: jax.Array,
    B_w1: jax.Array,
    B_b1: jax.Array,
    B_w2: jax.Array,
    B_b2: jax.Array,
    c: jax.Array,
    w_mod: jax.Array,
):
    del B_x
    any_spec = pl.BlockSpec(memory_space=pl.ANY)
    scratch = [
        pltpu.VMEM((_S, _D), _bf),
        pltpu.VMEM((_D, 3 * _D), _bf),
        pltpu.VMEM((_D, _D), _bf),
        pltpu.VMEM((_D, _F), _bf),
        pltpu.VMEM((1, _F), _bf),
        pltpu.VMEM((_F, _D), _bf),
        pltpu.VMEM((1, _D), _bf),
        pltpu.VMEM((1, _D), _bf),
        pltpu.VMEM((_D, 6 * _D), _bf),
        pltpu.VMEM((_D // 2, _D), _i32),
        pltpu.VMEM((_D // 2, _D), _i32),
        pltpu.VMEM((8, 6 * _D), _f32),
        pltpu.VMEM((4, _S // 2, 128), _i32),
        pltpu.VMEM((_NI, 128 // 2, _TQ), _i32),
        pltpu.VMEM((_H, _DH // 2, _S), _i32),
        pltpu.VMEM((_S, _TQ), _f32),
        pltpu.VMEM((_S, _TQ), _f32),
        pltpu.VMEM((_NI, _DH, _TQ), _f32),
        pltpu.VMEM((_S, _D), _bf),
        pltpu.SemaphoreType.DMA((17,)),
    ]
    return pl.pallas_call(
        _kernel,
        out_shape=jax.ShapeDtypeStruct((1, _S, _D), _bf),
        in_specs=[any_spec] * 9,
        out_specs=any_spec,
        scratch_shapes=scratch,
        compiler_params=pltpu.CompilerParams(vmem_limit_bytes=110 * 1024 * 1024),
        name="adaln_block",
    )(A_x, A_wqkv, A_wo, B_w1, B_b1.reshape(1, _F), B_w2, B_b2.reshape(1, _D), c, w_mod)
```

```python
import jax
import jax.numpy as jnp
import jax.experimental.pallas as pl
import jax.experimental.pallas.tpu as pltpu
from jax import lax

_S = 2048
_D = 512
_H = 32
_DH = 16
_F = 1792
_TQ = 512
_NT = _S // _TQ
_C = 128
_NC = _S // _C
_NI = _NT * _H
_NB = 8
_FC = 128
_OUT_TILES = tuple((256 * i, 256) for i in range(8))
_EPS = 1e-5
_LOG2E = 1.4426950408889634

_bf = jnp.bfloat16
_f32 = jnp.float32
_i32 = jnp.int32
_NN = (((1,), (0,)), ((), ()))
_NTD = (((1,), (1,)), ((), ()))


def _ldb(x):
    return pltpu.bitcast(x, _bf)


def _stb(x):
    return pltpu.bitcast(x, _i32)


def _dot(a, b, dims=_NN):
    return lax.dot_general(a, b, dims, preferred_element_type=_f32)


def _layernorm(x):
    m = jnp.mean(x, axis=-1, keepdims=True)
    xc = x - m
    v = jnp.mean(xc * xc, axis=-1, keepdims=True)
    return xc * lax.rsqrt(v + _EPS)


def _kernel(x_hbm, wqkv_hbm, wo_hbm, w1_hbm, b1_hbm, w2_hbm, b2_hbm, c_hbm, wm_hbm,
            out_hbm,
            k_s, qm_s, vt_s, ot_s, out_v, x_v, wqkv_v, wo_v, wm_v,
            wqt_s, wvt_s, w1_v, w2_v, mod_s, b1_v, b2_v, c_v, sems, *s_bufs):
    def cp(src, dst, i):
        return pltpu.make_async_copy(src, dst, sems.at[i])

    c_cp = cp(c_hbm, c_v, 0)
    wma_cp = cp(wm_hbm.at[:, pl.ds(0, 2 * _D)], wm_v.at[:, pl.ds(0, 2 * _D)], 1)
    x_cps = [cp(x_hbm.at[0, pl.ds(b * _TQ, _TQ), :], x_v.at[pl.ds(b * _TQ, _TQ), :], 2 + b)
             for b in range(_NT)]
    wq_cp, wk_cp, wv_cp = [
        cp(wqkv_hbm.at[:, pl.ds(i * _D, _D)], wqkv_v.at[:, pl.ds(i * _D, _D)], (6, 22, 23)[i])
        for i in range(3)]
    wmb_cp = cp(wm_hbm.at[:, pl.ds(2 * _D, 4 * _D)], wm_v.at[:, pl.ds(2 * _D, 4 * _D)], 7)
    wo_cp = cp(wo_hbm, wo_v, 8)
    w1_cp = cp(w1_hbm, w1_v, 9)
    w2_cp = cp(w2_hbm, w2_v, 10)
    b1_cp = cp(b1_hbm, b1_v, 11)
    b2_cp = cp(b2_hbm, b2_v, 12)
    out_cps = [cp(out_v.at[pl.ds(r0, nr), :], out_hbm.at[0, pl.ds(r0, nr), :], 13 + i)
               for i, (r0, nr) in enumerate(_OUT_TILES)]

    c_cp.start()
    wma_cp.start()
    x_cps[0].start()
    wk_cp.start()

    st = {}

    def phase0():
        qm_s[...] = jnp.zeros(qm_s.shape, _i32)
        c_cp.wait()
        cf = c_v[...].astype(_f32)
        sc = (cf * (1.0 / (1.0 + jnp.exp(-cf)))).astype(_bf)
        st["sc8"] = jnp.broadcast_to(sc, (16, _D))
        wma_cp.wait()
        x_cps[1].start()
        x_cps[2].start()
        mod_s[:, pl.ds(0, 2 * _D)] = _dot(st["sc8"], wm_v[:, pl.ds(0, 2 * _D)])[0:8]

    def phase1():
        sa = mod_s[0:1, pl.ds(0, _D)]
        ca1 = 1.0 + mod_s[0:1, pl.ds(_D, _D)]
        qscale = _DH ** -0.5 * _LOG2E

        def norm_mod(b):
            xb = x_v[pl.ds(b * _TQ, _TQ), :].astype(_f32)
            return (_layernorm(xb) * ca1 + sa).astype(_bf)

        x_cps[0].wait()
        hb = norm_mod(0)
        wk_cp.wait()
        x_cps[3].start()
        wq_cp.start()
        wv_cp.start()

        def k_proj(b, hb):
            kb = _dot(hb, wqkv_v[:, pl.ds(_D, _D)])
            for g in range(4):
                k_s[g, pl.ds(b * _TQ // 2, _TQ // 2), :] = _stb(kb[:, g * 128:(g + 1) * 128].astype(_bf))

        def qv_proj(b, hb):
            qt = _dot(_ldb(wqt_s[...]), hb, _NTD) * qscale
            vt = _dot(_ldb(wvt_s[...]), hb, _NTD)
            for h in range(_H):
                qm_s[b * _H + h, pl.ds((h % 8) * _DH // 2, _DH // 2), :] = _stb(
                    qt[h * _DH:(h + 1) * _DH, :].astype(_bf))
                vt_s[h, :, pl.ds(b * _TQ, _TQ)] = _stb(vt[h * _DH:(h + 1) * _DH, :].astype(_bf))

        hs = [hb]
        k_proj(0, hb)
        x_cps[1].wait()
        hs.append(norm_mod(1))
        x_cps[2].wait()
        k_proj(1, hs[1])
        hs.append(norm_mod(2))
        x_cps[3].wait()
        wq_cp.wait()
        wv_cp.wait()
        wmb_cp.start()
        wo_cp.start()
        w1_cp.start()
        w2_cp.start()
        b1_cp.start()
        b2_cp.start()
        k_proj(2, hs[2])
        hs.append(norm_mod(3))
        wqt_s[...] = _stb(wqkv_v[:, pl.ds(0, _D)].astype(_f32).T.astype(_bf))
        wvt_s[...] = _stb(wqkv_v[:, pl.ds(2 * _D, _D)].astype(_f32).T.astype(_bf))
        k_proj(3, hs[3])
        for b in range(_NT):
            qv_proj(b, hs[b])

    def qk_chunk(n, s_ref, j):
        g = (n % _H) // 8
        s = _dot(_ldb(k_s[g, pl.ds(j * _C // 2, _C // 2), :]), _ldb(qm_s[n]))
        s_ref[pl.ds(j * _C, _C), :] = s
        return jnp.max(s.reshape(_C // 8, 8, _TQ), axis=0)

    def row_max(m8):
        return jnp.broadcast_to(jnp.max(m8, axis=0, keepdims=True), (8, _TQ))

    def qk_only(n, s_ref):
        m8 = None
        for j in range(_NC):
            mm = qk_chunk(n, s_ref, j)
            m8 = mm if m8 is None else jnp.maximum(m8, mm)
        return row_max(m8)

    def attn_steps(n0, ms, produce, res):
        m8 = [None] * _NB
        l8 = [None] * _NB
        acc = [None] * _NB
        ps = {}
        total = _NB * _NC
        for k in range(total + 1):
            if k < total:
                t, j = divmod(k, _NC)
                s = s_bufs[t][pl.ds(j * _C, _C), :]
                p = jnp.exp2(s.reshape(_C // 8, 8, _TQ) - ms[t][None])
                ll = jnp.sum(p, axis=0)
                ps[k] = p.reshape(_C, _TQ).astype(_bf)
                l8[t] = ll if l8[t] is None else l8[t] + ll
                if produce:
                    mm = qk_chunk(n0 + t + _NB, s_bufs[t], j)
                    m8[t] = mm if m8[t] is None else jnp.maximum(m8[t], mm)
                    if j == _NC - 1:
                        res.append(row_max(m8[t]))
            if k >= 1:
                t, j = divmod(k - 1, _NC)
                n = n0 + t
                a = _dot(_ldb(vt_s[n % _H, :, pl.ds(j * _C, _C)]), ps.pop(k - 1))
                acc[t] = a if acc[t] is None else acc[t] + a
                if j == _NC - 1:
                    ot_s[n] = acc[t] * (1.0 / jnp.sum(l8[t], axis=0, keepdims=True))
            yield

    def phase2():
        ms = tuple(qk_only(t, s_bufs[t]) for t in range(_NB))

        def attn_body(i, ms):
            res = []
            for _ in attn_steps(_NB * i, ms, True, res):
                pass
            return tuple(res)

        st["m"] = lax.fori_loop(0, _NI // _NB - 1, attn_body, ms)

    def phase3():
        wmb_cp.wait()
        wo_cp.wait()
        w1_cp.wait()
        w2_cp.wait()
        b1_cp.wait()
        b2_cp.wait()
        mod_s[:, pl.ds(2 * _D, 4 * _D)] = _dot(st["sc8"], wm_v[:, pl.ds(2 * _D, 4 * _D)])[0:8]
        ga = mod_s[0:1, pl.ds(2 * _D, _D)]
        sb = mod_s[0:1, pl.ds(3 * _D, _D)]
        cb1 = 1.0 + mod_s[0:1, pl.ds(4 * _D, _D)]
        gb = mod_s[0:1, pl.ds(5 * _D, _D)]

        def pre(i):
            r0, nr = _OUT_TILES[i]
            t, q0 = divmod(r0, _TQ)
            ot = ot_s[pl.ds(t * _H, _H), :, pl.ds(q0, nr)].reshape(_D, nr)
            a = _dot(ot.T.astype(_bf), wo_v[...])
            x1 = x_v[pl.ds(r0, nr), :].astype(_f32) + ga * a
            h2 = (_layernorm(x1) * cb1 + sb).astype(_bf)
            return x1, h2

        def ffn_steps(i, x1, h2):
            y = None
            b1 = b1_v[...].astype(_f32).reshape(1, _F)
            for c0 in range(0, _F, _FC):
                hid = _dot(h2, w1_v[:, pl.ds(c0, _FC)]) + b1[:, c0:c0 + _FC]
                r = jnp.maximum(hid, 0.0)
                yield
                yy = _dot((r * r).astype(_bf), w2_v[pl.ds(c0, _FC), :])
                y = yy if y is None else y + yy
                yield
            y = y + b2_v[...].astype(_f32).reshape(1, _D)
            out_v[pl.ds(*_OUT_TILES[i]), :] = (x1 + gb * y).astype(out_v.dtype)
            out_cps[i].start()

        side = attn_steps(_NI - _NB, st["m"], False, None)
        n_out = len(_OUT_TILES)
        cur = pre(0)
        for i in range(n_out):
            steps = ffn_steps(i, *cur)
            if i + 1 < n_out and _OUT_TILES[i + 1][0] == (_NT - 1) * _TQ:
                for _ in side:
                    next(steps)
            nxt = pre(i + 1) if i + 1 < n_out else None
            for _ in steps:
                next(side, None)
            cur = nxt
        for i in range(n_out):
            out_cps[i].wait()

    phase0()
    phase1()
    phase2()
    phase3()


@jax.jit
def pallas_adaLN_cond__mha_block__dense_activation_squared_relu__prompt_kernel(
    A_x: jax.Array,
    A_wqkv: jax.Array,
    A_wo: jax.Array,
    B_x: jax.Array,
    B_w1: jax.Array,
    B_b1: jax.Array,
    B_w2: jax.Array,
    B_b2: jax.Array,
    c: jax.Array,
    w_mod: jax.Array,
):
    del B_x
    any_spec = pl.BlockSpec(memory_space=pl.ANY)
    scratch = [
        pltpu.VMEM((4, _S // 2, 128), _i32),
        pltpu.VMEM((_NI, 128 // 2, _TQ), _i32),
        pltpu.VMEM((_H, _DH // 2, _S), _i32),
        pltpu.VMEM((_NI, _DH, _TQ), _f32),
        pltpu.VMEM((_S, _D), _bf),
        pltpu.VMEM((_S, _D), _bf),
        pltpu.VMEM((_D, 3 * _D), _bf),
        pltpu.VMEM((_D, _D), _bf),
        pltpu.VMEM((_D, 6 * _D), _bf),
        pltpu.VMEM((_D // 2, _D), _i32),
        pltpu.VMEM((_D // 2, _D), _i32),
        pltpu.VMEM((_D, _F), _bf),
        pltpu.VMEM((_F, _D), _bf),
        pltpu.VMEM((8, 6 * _D), _f32),
        pltpu.VMEM((_F,), _bf),
        pltpu.VMEM((_D,), _bf),
        pltpu.VMEM((1, _D), _bf),
        pltpu.SemaphoreType.DMA((24,)),
    ] + [pltpu.VMEM((_S, _TQ), _f32)] * _NB
    return pl.pallas_call(
        _kernel,
        out_shape=jax.ShapeDtypeStruct((1, _S, _D), _bf),
        in_specs=[any_spec] * 9,
        out_specs=any_spec,
        scratch_shapes=scratch,
        compiler_params=pltpu.CompilerParams(vmem_limit_bytes=110 * 1024 * 1024),
        name="adaln_block",
    )(A_x, A_wqkv, A_wo, B_w1, B_b1, B_w2, B_b2, c, w_mod)
```
